```python
import jax
import jax.numpy as jnp

def _softmax(x, axis=-1):
    return jax.nn.softmax(x, axis=axis)
def _gelu(x):
    return jax.nn.gelu(x, approximate=True)
def _silu(x):
    return jax.nn.silu(x)
def _sigmoid(x):
    return jax.nn.sigmoid(x)
def _layernorm(x, axis=-1, eps=1e-5):
    m = jnp.mean(x, axis=axis, keepdims=True)
    v = jnp.var(x, axis=axis, keepdims=True)
    return (x - m) / jnp.sqrt(v + eps)
def _scatter_add(tgt, idx, src, axis=0):
    return tgt.at[idx].add(src)
def _segment_sum(src, seg, n):
    return jax.ops.segment_sum(src, seg, n)
class _Rng:
    def __init__(self, key):
        self._k = key
    def _next(self):
        self._k, sub = jax.random.split(self._k)
        return sub
    def normal(self, shape):
        return jax.random.normal(self._next(), shape, dtype=jnp.bfloat16)
    def randint(self, lo, hi, shape):
        return jax.random.randint(self._next(), shape, lo, hi, dtype=jnp.int32)
    def uniform(self, shape, lo=0.0, hi=1.0):
        return jax.random.uniform(self._next(), shape, jnp.bfloat16, lo, hi)
    def permutation(self, n):
        return jax.random.permutation(self._next(), n)


kernel_name = 'standalone__fft_conv__vision'

def setup_inputs():
    _rng = _Rng(jax.random.key(int.from_bytes(__import__("os").urandom(4), "little")))
    _w = (lambda a: (lambda t: t.astype(jnp.bfloat16) if jnp.issubdtype(t.dtype, jnp.floating) else t)(jnp.asarray(a)))
    H = W = 224
    C = 96
    K = 7
    return {
        "x": _w((lambda *s: _rng.normal(s) * 0.05)(1, H, W, C)),
        "w": _w((lambda *s: _rng.normal(s) * 0.05)(K, K, C, C)),
    }

def reference(x, w):
    B, H, W, C = x.shape
    K = w.shape[0]
    wp = jnp.pad(w, ((0, H - K), (0, W - K), (0, 0), (0, 0)))
    Xf = (lambda x, axes=(-2,-1): jnp.fft.rfft2(x.astype(jnp.float32), axes=axes))(x, axes=(1, 2))
    Wf = (lambda x, axes=(-2,-1): jnp.fft.rfft2(x.astype(jnp.float32), axes=axes))(wp, axes=(0, 1))
    Yf = jnp.einsum('bhwi,hwio->bhwo', Xf, Wf)
    y = (lambda x, s, axes=(-2,-1): jnp.fft.irfft2(x, s=s, axes=axes).astype(jnp.bfloat16))(Yf, (H, W), axes=(1, 2))
    return y
```

```python
import numpy as np
import jax
import jax.numpy as jnp
from jax import lax
import jax.experimental.pallas as pl
import jax.experimental.pallas.tpu as pltpu

H = W = 224
C = 96
T = 62
V = 56
NS = 31
HB = 32
NB = H // HB
PR = 2 * (8 + H)


def _consts():
    F = np.zeros((128, 128), np.float64)
    G = np.zeros((112, 128), np.float64)
    for tl in range(2):
        for s in range(NS):
            for n in range(T):
                k = 56 * tl + 10 + n
                if s == 0:
                    F[tl * 32 + s, k] = 1.0
                    F[64 + tl * 32 + s, k] = (-1.0) ** n
                else:
                    ph = 2 * np.pi * s * n / T
                    F[tl * 32 + s, k] = np.cos(ph)
                    F[64 + tl * 32 + s, k] = -np.sin(ph)
            for m in range(V):
                n = m + 6 - 3
                r = tl * V + m
                c = tl * 64 + 2 * s
                if s == 0:
                    G[r, c] = (-1.0) ** n / T
                    G[r, c + 1] = 1.0 / T
                else:
                    ph = 2 * np.pi * s * n / T
                    G[r, c] = 2 * np.cos(ph) / T
                    G[r, c + 1] = -2 * np.sin(ph) / T
    return F.astype(np.float32), G.astype(np.float32)


_F, _G = _consts()
_COS = [[float(np.cos(2 * np.pi * f * k / T)) for k in range(4)] for f in range(16)]
_SIN = [[float(np.sin(2 * np.pi * f * k / T)) for k in range(4)] for f in range(16)]

bf16 = jnp.bfloat16
f32 = jnp.float32
u32 = jnp.uint32


def _kernel(x_ref, xh_ref, w_ref, f_ref, g_ref, o_ref, p_ref, wt_ref, sd_ref, z_ref):
    step = pl.program_id(0)

    def fwd_row(xrow, prow):
        xr = xrow[...]
        for u in range(2):
            if u == 0:
                win = jnp.concatenate([xr[:, 208:224], xr[:, 0:112]], axis=1)
            else:
                win = xr[:, 96:224]
            win = jnp.concatenate([win, jnp.zeros((32, 128), bf16)], axis=0)
            r = lax.dot_general(f_ref[...], win, (((1,), (1,)), ((), ())), preferred_element_type=f32)
            b0, b1, c0, c1 = r[0:32], r[32:64], r[64:96], r[96:128]
            comps = (
                pltpu.pack_elementwise([b0 + c0, b1 + c1], packed_dtype=bf16),
                pltpu.pack_elementwise([b0, b1], packed_dtype=bf16),
                pltpu.pack_elementwise([c0, c1], packed_dtype=bf16),
            )
            for g in range(3):
                p_ref[pl.ds(g * 32 * PR + prow + u, 32, stride=PR), :] = comps[g]

    @pl.when(step == 0)
    def _init():
        with jax.named_scope("init"):
            z_ref[pl.ds(31, 128, stride=32), :] = jnp.zeros((128, 128), u32)
            for p in range(7):
                ws = []
                for k in range(7):
                    v = w_ref[p * 7 + k].astype(f32)
                    v = jnp.concatenate([v, jnp.zeros((C, 32), f32)], axis=1)
                    v = jnp.concatenate([v, jnp.zeros((32, 128), f32)], axis=0)
                    ws.append(v.T[:C])
                sd_ref[p * 7] = ws[3]
                for k in range(1, 4):
                    sd_ref[p * 7 + k] = ws[3 + k] + ws[3 - k]
                    sd_ref[p * 7 + 3 + k] = ws[3 + k] - ws[3 - k]

            def wgen(i, c):
                p = i // 6
                r0 = pl.multiple_of((i % 6) * 16, 16)
                rows = pl.ds(r0, 16)
                w0, s1, s2, s3, d1, d2, d3 = [sd_ref[p * 7 + k, rows, :] for k in range(7)]

                def put(s, g, val):
                    wt_ref[(s * 3 + g) * 7 + p, rows, :] = val.astype(bf16)

                put(0, 0, jnp.zeros((16, 128), f32))
                e = w0 + s2
                o = s1 + s3
                put(0, 1, e + o)
                put(0, 2, o - e)
                for f in range(1, 16):
                    cs, sn = _COS[f], _SIN[f]
                    a = w0 + s2 * cs[2]
                    b = s1 * cs[1] + s3 * cs[3]
                    cc = d2 * (-sn[2])
                    dd = d1 * (-sn[1]) + d3 * (-sn[3])
                    wr0, wr1 = a + b, a - b
                    wi0, wi1 = cc + dd, dd - cc
                    put(f, 0, wr0)
                    put(f, 1, wi0 - wr0)
                    put(f, 2, wr0 + wi0)
                    put(31 - f, 0, wr1)
                    put(31 - f, 1, wi1 - wr1)
                    put(31 - f, 2, wr1 + wi1)
                return c

            lax.fori_loop(0, 42, wgen, 0)
            for hl in range(8):
                fwd_row(xh_ref.at[hl], 2 * hl)

    with jax.named_scope("fwd"):
        base = step * (2 * HB) + 16
        for hl in range(HB):
            fwd_row(x_ref.at[hl], base + 2 * hl)

    with jax.named_scope("main"):
        def slot(s):
            ks = []
            for g in range(3):
                pb = (g * 32 + s) * PR + base
                rhs = jnp.concatenate(
                    [pltpu.bitcast(p_ref[pl.ds(pb - 2 * p, 2 * HB), :], bf16) for p in range(7)], axis=1)
                lhs = jnp.concatenate([wt_ref[(s * 3 + g) * 7 + p] for p in range(7)], axis=1)
                ks.append(lax.dot_general(lhs, rhs, (((1,), (1,)), ((), ())), preferred_element_type=f32))
            z = pltpu.pack_elementwise([ks[0] - ks[2], ks[0] + ks[1]], packed_dtype=bf16)
            z = jnp.concatenate([z, jnp.zeros((32, 128), u32)], axis=0)
            z_ref[pl.ds(s, 128, stride=32), :] = z.T

        for s in range(NS):
            slot(s)

    with jax.named_scope("inv"):
        for hl in range(HB):
            ys = []
            for u in range(2):
                zz = pltpu.bitcast(z_ref[pl.ds((2 * hl + u) * 64, 64), :], bf16)
                ys.append(jnp.dot(g_ref[...], zz, preferred_element_type=f32).astype(bf16))
            y = jnp.concatenate(ys + [jnp.zeros((32, 128), bf16)], axis=0)
            o_ref[hl] = y.T[:C, :W]


@jax.jit
def pallas_standalone__fft_conv__vision_kernel(x, w):
    x3 = x.reshape(H, W, C).transpose(0, 2, 1)
    w3 = w.reshape(49, C, C)
    fm = jnp.asarray(_F, dtype=bf16)
    gm = jnp.asarray(_G, dtype=bf16)
    y = pl.pallas_call(
        _kernel,
        grid=(NB,),
        in_specs=[
            pl.BlockSpec((HB, C, W), lambda i: (i, 0, 0)),
            pl.BlockSpec((8, C, W), lambda i: (27, 0, 0)),
            pl.BlockSpec((49, C, C), lambda i: (0, 0, 0)),
            pl.BlockSpec((128, 128), lambda i: (0, 0)),
            pl.BlockSpec((112, 128), lambda i: (0, 0)),
        ],
        out_specs=pl.BlockSpec((HB, C, W), lambda i: (i, 0, 0)),
        out_shape=jax.ShapeDtypeStruct((H, C, W), bf16),
        scratch_shapes=[
            pltpu.VMEM((3 * 32 * PR, 128), u32),
            pltpu.VMEM((NS * 3 * 7, C, 128), bf16),
            pltpu.VMEM((49, C, 128), f32),
            pltpu.VMEM((128 * 32, 128), u32),
        ],
        compiler_params=pltpu.CompilerParams(
            dimension_semantics=("arbitrary",), vmem_limit_bytes=100 * 2**20),
    )(x3, x3, w3, fm, gm)
    return y.transpose(0, 2, 1).reshape(1, H, W, C)
```

```python
import numpy as np
import jax
import jax.numpy as jnp
from jax import lax
import jax.experimental.pallas as pl
import jax.experimental.pallas.tpu as pltpu

H = W = 224
C = 96
T = 34
V = 28
NC = 16
NS = 17
HB = 32
JB = HB // 2
NB = H // HB
PR = 4 * (4 + H // 2) + 4
ZR = 20
NT = 11

bf16 = jnp.bfloat16
f32 = jnp.float32
u32 = jnp.uint32


def _pack_rows(m):
    b = np.asarray(m, np.float32).view(np.uint32).astype(np.uint64)
    b = ((b + 0x7FFF + ((b >> 16) & 1)) >> 16).astype(np.uint32)
    return (b[0::2] | (b[1::2] << 16)).astype(np.uint32)


def _consts():
    F = np.zeros((2, 144, 128), np.float64)
    G = np.zeros((64, 128), np.float64)
    for u in range(2):
        if u == 0:
            wl = [l if l < 112 else l + 96 for l in range(128)]
        else:
            wl = [128 + l if l < 96 else l for l in range(128)]
        for tl in range(4):
            t = 4 * u + tl
            for l in range(128):
                n = (wl[l] - (V * t - 6)) % W
                if n >= T:
                    continue
                for s in range(NC):
                    ph = 2 * np.pi * (s + 1) * n / T
                    F[u, tl * 16 + s, l] = np.cos(ph)
                    F[u, 64 + tl * 16 + s, l] = -np.sin(ph)
                r = 128 + 8 * (tl % 2) + tl // 2
                F[u, r, l] = 1.0
                F[u, r + 2, l] = (-1.0) ** n
    for tl in range(2):
        for m in range(V):
            n = m + 6 - 3
            r = tl * V + m
            for s in range(NC):
                ph = 2 * np.pi * (s + 1) * n / T
                G[r, tl * 2 * ZR + 2 * s] = 2 * np.cos(ph) / T
                G[r, tl * 2 * ZR + 2 * s + 1] = -2 * np.sin(ph) / T
            G[r, tl * 2 * ZR + 2 * NC] = (-1.0) ** n / T
            G[r, tl * 2 * ZR + 2 * NC + 1] = 1.0 / T
    return np.stack([_pack_rows(F[0]), _pack_rows(F[1])]), _pack_rows(G)


_F, _G = _consts()
_COS = [[float(np.cos(2 * np.pi * f * k / T)) for k in range(4)] for f in range(9)]
_SIN = [[float(np.sin(2 * np.pi * f * k / T)) for k in range(4)] for f in range(9)]
_NT_DIMS = (((1,), (1,)), ((), ()))


def _kernel(x_ref, xh_ref, w_ref, f_ref, g_ref, o_ref, p_ref, pr_ref, wt_ref, sd_ref, z_ref, rp_ref):
    step = pl.program_id(0)

    def dft(xrow, u):
        xr = xrow[...]
        if u == 0:
            win = jnp.concatenate([xr[:, 0:112], xr[:, 208:224]], axis=1)
        else:
            win = jnp.concatenate([xr[:, 128:224], xr[:, 96:128]], axis=1)
        win = jnp.concatenate([win, jnp.zeros((32, 128), bf16)], axis=0)
        return lax.dot_general(pltpu.bitcast(f_ref[u], bf16), win, _NT_DIMS, preferred_element_type=f32)

    def emit(r, m, row):
        pk = lambda a, b: pltpu.pack_elementwise([a, b], packed_dtype=bf16)
        for pp in range(2):
            b0, b1 = r[32 * pp:32 * pp + 16], r[32 * pp + 16:32 * pp + 32]
            c0, c1 = r[64 + 32 * pp:64 + 32 * pp + 16], r[64 + 32 * pp + 16:64 + 32 * pp + 32]
            comps = (pk(b0 + c0, b1 + c1), pk(b0, b1), pk(c0, c1))
            for g in range(3):
                p_ref[pl.ds((m * 3 + g) * NC * PR + row + pp, NC, stride=PR), :] = comps[g]
        rr = pk(r[128:136], r[136:144])
        for c in range(2):
            pr_ref[pl.ds((m * 2 + c) * PR + row, 2), :] = rr[2 * c:2 * c + 2]

    def fwd_pairs(src, h0, npairs, row0, u, prev):
        for jj in range(npairs):
            r0 = dft(src.at[h0 + 2 * jj], u)
            r1 = dft(src.at[h0 + 2 * jj + 1], u)
            row = row0 + 4 * jj + 2 * u
            emit(r0, 0, row)
            emit(r1 - r0, 1, row)
            if prev is not None:
                emit(r0 - prev, 2, row)
            prev = r1
        return prev

    @pl.when(step == 0)
    def _init():
        with jax.named_scope("init"):
            z_ref[...] = jnp.zeros(z_ref.shape, u32)
            for kw in range(7):
                ws = []
                for p in range(7):
                    v = w_ref[p * 7 + kw].astype(f32)
                    v = jnp.concatenate([v, jnp.zeros((C, 32), f32)], axis=1)
                    v = jnp.concatenate([v, jnp.zeros((32, 128), f32)], axis=0)
                    ws.append(v.T[:C])
                for q in range(4):
                    sd_ref[q * 7 + kw] = ws[2 * q] + ws[2 * q + 1] if q < 3 else ws[6]
                    sd_ref[(4 + q) * 7 + kw] = ws[2 * q]
                    if q < 3:
                        sd_ref[(8 + q) * 7 + kw] = -ws[2 * q + 1]

            def wgen(i, c):
                tp = i // 6
                r0 = pl.multiple_of((i % 6) * 16, 16)
                rows = pl.ds(r0, 16)
                t_ = [sd_ref[tp * 7 + k, rows, :] for k in range(7)]
                w0 = t_[3]
                s1, s2, s3 = t_[4] + t_[2], t_[5] + t_[1], t_[6] + t_[0]
                d1, d2, d3 = t_[4] - t_[2], t_[5] - t_[1], t_[6] - t_[0]

                def put(s, g, val):
                    wt_ref[(s * 3 + g) * NT + tp, rows, :] = val.astype(bf16)

                e = w0 + s2
                o = s1 + s3
                put(NC, 1, e + o)
                put(NC, 2, e - o)
                for f in range(1, 9):
                    cs, sn = _COS[f], _SIN[f]
                    a = w0 + s2 * cs[2]
                    b = s1 * cs[1] + s3 * cs[3]
                    cc = d2 * (-sn[2])
                    dd = d1 * (-sn[1]) + d3 * (-sn[3])
                    wr0, wr1 = a + b, a - b
                    wi0, wi1 = cc + dd, dd - cc
                    put(f - 1, 0, wr0)
                    put(f - 1, 1, wi0 - wr0)
                    put(f - 1, 2, wr0 + wi0)
                    put(16 - f, 0, wr1)
                    put(16 - f, 1, wi1 - wr1)
                    put(16 - f, 2, wr1 + wi1)
                return c

            lax.fori_loop(0, NT * 6, wgen, 0)
            for u in range(2):
                rp_ref[u] = fwd_pairs(xh_ref, 0, 4, 0, u, None)

    with jax.named_scope("fwd"):
        base = step * (4 * JB) + 16
        for u in range(2):
            rp_ref[u] = fwd_pairs(x_ref, 0, JB, base, u, rp_ref[u])

    with jax.named_scope("main"):
        def prod(src, sb, wb, m):
            nt, t0 = ((4, 0), (4, 4), (3, 8))[m]
            rhs = jnp.concatenate(
                [pltpu.bitcast(src[pl.ds(sb + base - 4 * q, 4 * JB), :], bf16) for q in range(nt)], axis=1)
            lhs = jnp.concatenate([wt_ref[wb + t0 + q] for q in range(nt)], axis=1)
            return lax.dot_general(lhs, rhs, _NT_DIMS, preferred_element_type=f32)

        def put_z(yr, yi, e, s):
            z = pltpu.pack_elementwise([yr, yi], packed_dtype=bf16)
            zt = jnp.concatenate([z, jnp.zeros((32, 128), u32)], axis=0).T
            for j in range(JB):
                z_ref[pl.ds((2 * j + e) * 8 * ZR + s, 8, stride=ZR), :] = zt[8 * j:8 * j + 8]

        for s in range(NS):
            ms = []
            for m in range(3):
                if s < NC:
                    k = [prod(p_ref, ((m * 3 + g) * NC + s) * PR, (s * 3 + g) * NT, m) for g in range(3)]
                    ms.append((k[0] - k[2], k[0] + k[1]))
                else:
                    ms.append((prod(pr_ref, (m * 2 + 1) * PR, (s * 3 + 2) * NT, m),
                               prod(pr_ref, (m * 2) * PR, (s * 3 + 1) * NT, m)))
                if m == 1:
                    put_z(ms[0][0] + ms[1][0], ms[0][1] + ms[1][1], 1, s)
            put_z(ms[0][0] + ms[2][0], ms[0][1] + ms[2][1], 0, s)

    with jax.named_scope("inv"):
        for hl in range(HB):
            ys = []
            for q in range(4):
                zz = pltpu.bitcast(z_ref[pl.ds((hl * 8 + 2 * q) * ZR, 2 * ZR), :], bf16)
                zz = jnp.concatenate([zz, jnp.zeros((128 - 4 * ZR, 128), bf16)], axis=0)
                y = jnp.dot(pltpu.bitcast(g_ref[...], bf16), zz, preferred_element_type=f32)
                ys.append(y[:2 * V])
            y = jnp.concatenate(ys + [jnp.zeros((32, 128), f32)], axis=0)
            o_ref[hl] = y.T[:C, :W].astype(bf16)


@jax.jit
def pallas_standalone__fft_conv__vision_kernel(x, w):
    x3 = x.reshape(H, W, C).transpose(0, 2, 1)
    w3 = w.reshape(49, C, C)
    fm = jnp.asarray(_F)
    gm = jnp.asarray(_G)
    y = pl.pallas_call(
        _kernel,
        grid=(NB,),
        in_specs=[
            pl.BlockSpec((HB, C, W), lambda i: (i, 0, 0)),
            pl.BlockSpec((8, C, W), lambda i: (27, 0, 0)),
            pl.BlockSpec((49, C, C), lambda i: (0, 0, 0)),
            pl.BlockSpec((2, 72, 128), lambda i: (0, 0, 0)),
            pl.BlockSpec((32, 128), lambda i: (0, 0)),
        ],
        out_specs=pl.BlockSpec((HB, C, W), lambda i: (i, 0, 0)),
        out_shape=jax.ShapeDtypeStruct((H, C, W), bf16),
        scratch_shapes=[
            pltpu.VMEM((9 * NC * PR, 128), u32),
            pltpu.VMEM((6 * PR + 4, 128), u32),
            pltpu.VMEM((NS * 3 * NT, C, 128), bf16),
            pltpu.VMEM((NT * 7, C, 128), f32),
            pltpu.VMEM((HB * 8 * ZR, 128), u32),
            pltpu.VMEM((2, 144, 128), f32),
        ],
        compiler_params=pltpu.CompilerParams(
            dimension_semantics=("arbitrary",), vmem_limit_bytes=100 * 2**20),
    )(x3, x3, w3, fm, gm)
    return y.transpose(0, 2, 1).reshape(1, H, W, C)
```

```python
import numpy as np
import jax
import jax.numpy as jnp
from jax import lax
import jax.experimental.pallas as pl
import jax.experimental.pallas.tpu as pltpu

H = W = 224
C = 96
T = 34
V = 28
NC = 16
NS = 17
HB = 32
JB = HB // 2
NB = H // HB
PR = 4 * (4 + H // 2) + 4
ZR = 20
NT = 9

bf16 = jnp.bfloat16
f32 = jnp.float32
u32 = jnp.uint32


def _pack_rows(m):
    b = np.asarray(m, np.float32).view(np.uint32).astype(np.uint64)
    b = ((b + 0x7FFF + ((b >> 16) & 1)) >> 16).astype(np.uint32)
    return (b[0::2] | (b[1::2] << 16)).astype(np.uint32)


def _consts():
    F = np.zeros((2, 144, 128), np.float64)
    G = np.zeros((64, 128), np.float64)
    for u in range(2):
        if u == 0:
            wl = [l if l < 112 else l + 96 for l in range(128)]
        else:
            wl = [128 + l if l < 96 else l for l in range(128)]
        for tl in range(4):
            t = 4 * u + tl
            for l in range(128):
                n = (wl[l] - (V * t - 6)) % W
                if n >= T:
                    continue
                for s in range(NC):
                    ph = 2 * np.pi * (s + 1) * n / T
                    F[u, tl * 16 + s, l] = np.cos(ph)
                    F[u, 64 + tl * 16 + s, l] = -np.sin(ph)
                r = 128 + 8 * (tl % 2) + tl // 2
                F[u, r, l] = 1.0
                F[u, r + 2, l] = (-1.0) ** n
    for tl in range(2):
        for m in range(V):
            n = m + 6 - 3
            r = tl * V + m
            for s in range(NC):
                ph = 2 * np.pi * (s + 1) * n / T
                G[r, tl * 2 * ZR + 2 * s] = 2 * np.cos(ph) / T
                G[r, tl * 2 * ZR + 2 * s + 1] = -2 * np.sin(ph) / T
            G[r, tl * 2 * ZR + 2 * NC] = (-1.0) ** n / T
            G[r, tl * 2 * ZR + 2 * NC + 1] = 1.0 / T
    return np.stack([_pack_rows(F[0]), _pack_rows(F[1])]), _pack_rows(G)


_F, _G = _consts()
_COS = [[float(np.cos(2 * np.pi * f * k / T)) for k in range(4)] for f in range(9)]
_SIN = [[float(np.sin(2 * np.pi * f * k / T)) for k in range(4)] for f in range(9)]
_NT_DIMS = (((1,), (1,)), ((), ()))


def _kernel(x_ref, xh_ref, w_ref, f_ref, g_ref, o_ref, p_ref, pr_ref, wt_ref, sd_ref, z_ref, rp_ref):
    step = pl.program_id(0)

    def dft(xrow, u):
        xr = xrow[...]
        if u == 0:
            win = jnp.concatenate([xr[:, 0:112], xr[:, 208:224]], axis=1)
        else:
            win = jnp.concatenate([xr[:, 128:224], xr[:, 96:128]], axis=1)
        win = jnp.concatenate([win, jnp.zeros((32, 128), bf16)], axis=0)
        return lax.dot_general(pltpu.bitcast(f_ref[u], bf16), win, _NT_DIMS, preferred_element_type=f32)

    def emit(r, m, row):
        pk = lambda a, b: pltpu.pack_elementwise([a, b], packed_dtype=bf16)
        for pp in range(2):
            b0, b1 = r[32 * pp:32 * pp + 16], r[32 * pp + 16:32 * pp + 32]
            c0, c1 = r[64 + 32 * pp:64 + 32 * pp + 16], r[64 + 32 * pp + 16:64 + 32 * pp + 32]
            comps = (pk(b0 + c0, b1 + c1), pk(b0, b1), pk(c0, c1))
            for g in range(3):
                p_ref[pl.ds((m * 3 + g) * NC * PR + row + pp, NC, stride=PR), :] = comps[g]
        rr = pk(r[128:136], r[136:144])
        for c in range(2):
            pr_ref[pl.ds((m * 2 + c) * PR + row, 2), :] = rr[2 * c:2 * c + 2]

    def fwd_pairs(src, h0, npairs, row0, u, prev):
        for jj in range(npairs):
            r0 = dft(src.at[h0 + 2 * jj], u)
            r1 = dft(src.at[h0 + 2 * jj + 1], u)
            row = row0 + 4 * jj + 2 * u
            emit(r0, 0, row)
            emit(r1 - r0, 1, row)
            if prev is not None:
                emit(r0 - prev, 2, row)
            prev = r1
        return prev

    @pl.when(step == 0)
    def _init():
        with jax.named_scope("init"):
            z_ref[...] = jnp.zeros(z_ref.shape, u32)
            for kw in range(7):
                ws = [w_ref[p * 7 + kw].astype(f32) for p in range(7)]
                seqs = ([ws[0] + ws[1], ws[2] + ws[3], ws[4] + ws[5], ws[6]],
                        [ws[0], ws[2], ws[4], ws[6]])
                tiles = []
                for sq in seqs:
                    d = jnp.concatenate(sq, axis=0)
                    tiles += [d[128 * k:128 * (k + 1)] for k in range(3)]
                for q in range(3):
                    tiles.append(jnp.concatenate([-ws[2 * q + 1], jnp.zeros((32, C), f32)], axis=0))
                for k, v in enumerate(tiles):
                    v = jnp.concatenate([v, jnp.zeros((128, 32), f32)], axis=1)
                    sd_ref[k * 7 + kw] = v.T[:C]

            def wgen(i, c):
                tp = i // 6
                r0 = pl.multiple_of((i % 6) * 16, 16)
                rows = pl.ds(r0, 16)
                t_ = [sd_ref[tp * 7 + k, rows, :] for k in range(7)]
                w0 = t_[3]
                s1, s2, s3 = t_[4] + t_[2], t_[5] + t_[1], t_[6] + t_[0]
                d1, d2, d3 = t_[4] - t_[2], t_[5] - t_[1], t_[6] - t_[0]

                def put(s, g, val):
                    wt_ref[(s * 3 + g) * NT + tp, rows, :] = val.astype(bf16)

                e = w0 + s2
                o = s1 + s3
                put(NC, 1, e + o)
                put(NC, 2, e - o)
                for f in range(1, 9):
                    cs, sn = _COS[f], _SIN[f]
                    a = w0 + s2 * cs[2]
                    b = s1 * cs[1] + s3 * cs[3]
                    cc = d2 * (-sn[2])
                    dd = d1 * (-sn[1]) + d3 * (-sn[3])
                    wr0, wr1 = a + b, a - b
                    wi0, wi1 = cc + dd, dd - cc
                    put(f - 1, 0, wr0)
                    put(f - 1, 1, wi0 - wr0)
                    put(f - 1, 2, wr0 + wi0)
                    put(16 - f, 0, wr1)
                    put(16 - f, 1, wi1 - wr1)
                    put(16 - f, 2, wr1 + wi1)
                return c

            lax.fori_loop(0, NT * 6, wgen, 0)
            for u in range(2):
                rp_ref[u] = fwd_pairs(xh_ref, 0, 4, 0, u, None)

    with jax.named_scope("fwd"):
        base = step * (4 * JB) + 16
        for u in range(2):
            rp_ref[u] = fwd_pairs(x_ref, 0, JB, base, u, rp_ref[u])

    with jax.named_scope("main"):
        lane = lax.broadcasted_iota(jnp.int32, (4 * JB, 128), 1)

        def prod(src, sb, wb, m):
            ld = lambda q: src[pl.ds(sb + base - 4 * q, 4 * JB), :]
            if m < 2:
                r1, r2, r3 = pltpu.roll(ld(1), 96, 1), pltpu.roll(ld(2), 64, 1), pltpu.roll(ld(3), 32, 1)
                parts = [jnp.where(lane < 96, ld(0), r1), jnp.where(lane < 64, r1, r2), jnp.where(lane < 32, r2, r3)]
            else:
                parts = [ld(0), ld(1), ld(2)]
            rhs = jnp.concatenate([pltpu.bitcast(v, bf16) for v in parts], axis=1)
            lhs = jnp.concatenate([wt_ref[wb + 3 * m + q] for q in range(3)], axis=1)
            return lax.dot_general(lhs, rhs, _NT_DIMS, preferred_element_type=f32)

        def put_z(yr, yi, e, s):
            z = pltpu.pack_elementwise([yr, yi], packed_dtype=bf16)
            zt = jnp.concatenate([z, jnp.zeros((32, 128), u32)], axis=0).T
            for j in range(JB):
                z_ref[pl.ds((2 * j + e) * 8 * ZR + s, 8, stride=ZR), :] = zt[8 * j:8 * j + 8]

        for s in range(NS):
            ms = []
            for m in range(3):
                if s < NC:
                    k = [prod(p_ref, ((m * 3 + g) * NC + s) * PR, (s * 3 + g) * NT, m) for g in range(3)]
                    ms.append((k[0] - k[2], k[0] + k[1]))
                else:
                    ms.append((prod(pr_ref, (m * 2 + 1) * PR, (s * 3 + 2) * NT, m),
                               prod(pr_ref, (m * 2) * PR, (s * 3 + 1) * NT, m)))
                if m == 1:
                    put_z(ms[0][0] + ms[1][0], ms[0][1] + ms[1][1], 1, s)
            put_z(ms[0][0] + ms[2][0], ms[0][1] + ms[2][1], 0, s)

    with jax.named_scope("inv"):
        for hl in range(HB):
            ys = []
            for q in range(4):
                zz = pltpu.bitcast(z_ref[pl.ds((hl * 8 + 2 * q) * ZR, 2 * ZR), :], bf16)
                zz = jnp.concatenate([zz, jnp.zeros((128 - 4 * ZR, 128), bf16)], axis=0)
                y = jnp.dot(pltpu.bitcast(g_ref[...], bf16), zz, preferred_element_type=f32)
                ys.append(y[:2 * V])
            y = jnp.concatenate(ys + [jnp.zeros((32, 128), f32)], axis=0)
            o_ref[hl] = y.T[:C, :W].astype(bf16)


@jax.jit
def pallas_standalone__fft_conv__vision_kernel(x, w):
    x3 = x.reshape(H, W, C).transpose(0, 2, 1)
    w3 = w.reshape(49, C, C)
    fm = jnp.asarray(_F)
    gm = jnp.asarray(_G)
    y = pl.pallas_call(
        _kernel,
        grid=(NB,),
        in_specs=[
            pl.BlockSpec((HB, C, W), lambda i: (i, 0, 0)),
            pl.BlockSpec((8, C, W), lambda i: (27, 0, 0)),
            pl.BlockSpec((49, C, C), lambda i: (0, 0, 0)),
            pl.BlockSpec((2, 72, 128), lambda i: (0, 0, 0)),
            pl.BlockSpec((32, 128), lambda i: (0, 0)),
        ],
        out_specs=pl.BlockSpec((HB, C, W), lambda i: (i, 0, 0)),
        out_shape=jax.ShapeDtypeStruct((H, C, W), bf16),
        scratch_shapes=[
            pltpu.VMEM((9 * NC * PR, 128), u32),
            pltpu.VMEM((6 * PR + 4, 128), u32),
            pltpu.VMEM((NS * 3 * NT, C, 128), bf16),
            pltpu.VMEM((NT * 7, C, 128), f32),
            pltpu.VMEM((HB * 8 * ZR, 128), u32),
            pltpu.VMEM((2, 144, 128), f32),
        ],
        compiler_params=pltpu.CompilerParams(
            dimension_semantics=("arbitrary",), vmem_limit_bytes=100 * 2**20),
    )(x3, x3, w3, fm, gm)
    return y.transpose(0, 2, 1).reshape(1, H, W, C)
```

```python
import numpy as np
import jax
import jax.numpy as jnp
from jax import lax
import jax.experimental.pallas as pl
import jax.experimental.pallas.tpu as pltpu

H = W = 224
C = 96
T = 34
V = 28
NC = 16
NS = 17
HB = 32
JB = HB // 2
NB = H // HB
PR = 4 * (4 + H // 2) + 4
ZR = 20
NT = 9

bf16 = jnp.bfloat16
f32 = jnp.float32
u32 = jnp.uint32


def _round_bf16(m):
    b = np.ascontiguousarray(m, np.float32).view(np.uint32).astype(np.uint64)
    b = ((b + 0x7FFF + ((b >> 16) & 1)) >> 16) << 16
    return b.astype(np.uint32).view(np.float32)


def _consts():
    fm = np.zeros((2, 136, 128), np.float64)
    gm = np.zeros((2 * V, 128), np.float64)
    for u in range(2):
        wl = [l if l < 112 else l + 96 for l in range(128)] if u == 0 else \
             [128 + l if l < 96 else l for l in range(128)]
        for tl in range(4):
            for l in range(128):
                n = (wl[l] - (V * (4 * u + tl) - 6)) % W
                if n >= T:
                    continue
                for s in range(NC):
                    ph = 2 * np.pi * (s + 1) * n / T
                    fm[u, tl * 16 + s, l] = np.cos(ph)
                    fm[u, 64 + tl * 16 + s, l] = -np.sin(ph)
                r = 128 + 4 * (tl % 2) + tl // 2
                fm[u, r, l] = 1.0
                fm[u, r + 2, l] = (-1.0) ** n
    for tl in range(2):
        for m in range(V):
            n = m + 6 - 3
            r, c = tl * V + m, tl * 2 * ZR
            for s in range(NC):
                ph = 2 * np.pi * (s + 1) * n / T
                gm[r, c + 2 * s] = 2 * np.cos(ph) / T
                gm[r, c + 2 * s + 1] = -2 * np.sin(ph) / T
            gm[r, c + 2 * NC] = (-1.0) ** n / T
            gm[r, c + 2 * NC + 1] = 1.0 / T
    return _round_bf16(fm), _round_bf16(gm)


_F, _G = _consts()
_COS = [[float(np.cos(2 * np.pi * f * k / T)) for k in range(4)] for f in range(9)]
_SIN = [[float(np.sin(2 * np.pi * f * k / T)) for k in range(4)] for f in range(9)]
_NT_DIMS = (((1,), (1,)), ((), ()))
_NN_DIMS = (((1,), (0,)), ((), ()))


def _pk(lo, hi):
    return pltpu.pack_elementwise([lo, hi], packed_dtype=bf16)


def _kernel(x_hbm, w_hbm, f_ref, g_ref, o_hbm,
            p_ref, pr_ref, wt_ref, sd_ref, z_ref, rp_ref, xb_ref, xh_ref, w_ref, ob_ref, isem, osem):
    w_cp = pltpu.make_async_copy(w_hbm, w_ref, isem.at[NB])
    h_cp = pltpu.make_async_copy(x_hbm.at[pl.ds(H - 8, 8)], xh_ref, isem.at[NB + 1])

    def x_cp(b):
        return pltpu.make_async_copy(x_hbm.at[pl.ds(b * HB, HB)], xb_ref.at[pl.ds(b * HB, HB)], isem.at[b])

    def o_cp(c):
        return pltpu.make_async_copy(ob_ref.at[pl.ds(c * 8, 8)], o_hbm.at[pl.ds(c * 8, 8)], osem.at[c])

    def dft(xrow, u):
        xr = xrow[...]
        if u == 0:
            win = jnp.concatenate([xr[:, 0:112], xr[:, 208:224]], axis=1)
        else:
            win = jnp.concatenate([xr[:, 128:224], xr[:, 96:128]], axis=1)
        win = jnp.concatenate([win, jnp.zeros((128 - C, 128), bf16)], axis=0)
        return lax.dot_general(f_ref[u], win, _NT_DIMS, preferred_element_type=f32)

    def emit(r, m, row):
        for pp in range(2):
            b0, b1 = r[32 * pp:32 * pp + 16], r[32 * pp + 16:32 * pp + 32]
            c0, c1 = r[64 + 32 * pp:80 + 32 * pp], r[80 + 32 * pp:96 + 32 * pp]
            for g, v in enumerate((_pk(b0 + c0, b1 + c1), _pk(b0, b1), _pk(c0, c1))):
                p_ref[pl.ds((m * 3 + g) * NC * PR + row + pp, NC, stride=PR), :] = v
        rr = _pk(r[128:136], pltpu.roll(r[128:136], 4, 0))
        for c in range(2):
            pr_ref[pl.ds((m * 2 + c) * PR + row, 2), :] = rr[2 * c:2 * c + 2]

    def fwd_rows(src, h0, npairs, row0, first):
        for u in range(2):
            prev = None if first else rp_ref[u]
            for jj in range(npairs):
                r0 = dft(src.at[h0 + 2 * jj], u)
                r1 = dft(src.at[h0 + 2 * jj + 1], u)
                row = row0 + 4 * jj + 2 * u
                emit(r0, 0, row)
                emit(r1 - r0, 1, row)
                if prev is not None:
                    emit(r0 - prev, 2, row)
                prev = r1
            rp_ref[u] = prev

    def fwd_block(b):
        fwd_rows(xb_ref, b * HB, JB, b * (4 * JB) + 16, False)

    def w_prep():
        for kw in range(7):
            ws = [w_ref[p * 7 + kw].astype(f32) for p in range(7)]
            tiles = []
            for sq in ([ws[0] + ws[1], ws[2] + ws[3], ws[4] + ws[5], ws[6]], [ws[0], ws[2], ws[4], ws[6]]):
                d = jnp.concatenate(sq, axis=0)
                tiles += [d[128 * k:128 * (k + 1)] for k in range(3)]
            for q in range(3):
                tiles.append(jnp.concatenate([-ws[2 * q + 1], jnp.zeros((128 - C, C), f32)], axis=0))
            for k, v in enumerate(tiles):
                v = jnp.concatenate([v, jnp.zeros((128, 128 - C), f32)], axis=1)
                sd_ref[k * 7 + kw] = v.T[:C]
        for tp in range(NT):
            t_ = [sd_ref[tp * 7 + k] for k in range(7)]
            sd_ref[tp * 7] = t_[3]
            for k in range(1, 4):
                sd_ref[tp * 7 + k] = t_[3 + k] + t_[3 - k]
                sd_ref[tp * 7 + 3 + k] = t_[3 + k] - t_[3 - k]

    def wgen_piece(f, k):
        tp, og = k // 6, k % 6
        outs = []
        for par in range(2):
            rows = pl.ds(16 * og + par, 8, stride=2)
            if f == 0:
                w0, s1, s2, s3 = [sd_ref[tp * 7 + i, rows, :] for i in range(4)]
                e, o = w0 + s2, s1 + s3
                outs.append((e + o, e - o))
                continue
            w0, s1, s2, s3, d1, d2, d3 = [sd_ref[tp * 7 + i, rows, :] for i in range(7)]
            cs, sn = _COS[f], _SIN[f]
            a, b = w0 + s2 * cs[2], s1 * cs[1] + s3 * cs[3]
            cc, dd = d2 * (-sn[2]), d1 * (-sn[1]) + d3 * (-sn[3])
            wr0, wr1, wi0, wi1 = a + b, a - b, cc + dd, dd - cc
            outs.append((wr0, wi0 - wr0, wr0 + wi0, wr1, wi1 - wr1, wr1 + wi1))
        dst = ((NC, 1), (NC, 2)) if f == 0 else \
              ((f - 1, 0), (f - 1, 1), (f - 1, 2), (16 - f, 0), (16 - f, 1), (16 - f, 2))
        for i, (s, g) in enumerate(dst):
            wt_ref[(s * 3 + g) * NT + tp, pl.ds(8 * og, 8), :] = _pk(outs[0][i], outs[1][i])

    def prod(src, sb, wb, m):
        lane = lax.broadcasted_iota(jnp.int32, (4 * JB, 128), 1)
        ld = lambda q: src[pl.ds(sb - 4 * q, 4 * JB), :]
        if m < 2:
            r1, r2, r3 = pltpu.roll(ld(1), 96, 1), pltpu.roll(ld(2), 64, 1), pltpu.roll(ld(3), 32, 1)
            parts = [jnp.where(lane < 96, ld(0), r1), jnp.where(lane < 64, r1, r2), jnp.where(lane < 32, r2, r3)]
        else:
            parts = [ld(0), ld(1), ld(2)]
        rhs = jnp.concatenate([pltpu.bitcast(v, bf16) for v in parts], axis=1)
        lhs = jnp.concatenate([pltpu.bitcast(wt_ref[wb + 3 * m + q], bf16) for q in range(3)], axis=1)
        return lax.dot_general(lhs, rhs, _NT_DIMS, preferred_element_type=f32)

    def put_z(yr, yi, e, s):
        zt = jnp.concatenate([_pk(yr, yi), jnp.zeros((128 - C, 128), u32)], axis=0).T
        for j in range(JB):
            z_ref[pl.ds((2 * j + e) * 8 * ZR + s, 8, stride=ZR), :] = zt[8 * j:8 * j + 8]

    def main_slot(b, s, side=None):
        base = b * (4 * JB) + 16
        ms = []
        for m in range(3):
            if s < NC:
                k = []
                for g in range(3):
                    k.append(prod(p_ref, ((m * 3 + g) * NC + s) * PR + base, (s * 3 + g) * NT, m))
                    if side is not None:
                        side(m * 3 + g)
                ms.append((k[0] - k[2], k[0] + k[1]))
            else:
                ms.append((prod(pr_ref, (m * 2 + 1) * PR + base, (s * 3 + 2) * NT, m),
                           prod(pr_ref, (m * 2) * PR + base, (s * 3 + 1) * NT, m)))
            if m == 1:
                put_z(ms[0][0] + ms[1][0], ms[0][1] + ms[1][1], 1, s)
        put_z(ms[0][0] + ms[2][0], ms[0][1] + ms[2][1], 0, s)

    def main_block(b):
        for s in range(NS):
            main_slot(b, s)

    def inv_row(b, hl):
        ys = []
        for q in range(4):
            zz = pltpu.bitcast(z_ref[pl.ds((hl * 8 + 2 * q) * ZR, 2 * ZR), :], bf16)
            zz = jnp.concatenate([zz, jnp.zeros((128 - 4 * ZR, 128), bf16)], axis=0)
            ys.append(lax.dot_general(g_ref[...], zz, _NN_DIMS, preferred_element_type=f32))
        y = jnp.concatenate(ys + [jnp.zeros((256 - W, 128), f32)], axis=0)
        ob_ref[b * HB + hl] = y.T[:C, :W].astype(bf16)

    def inv_block(b):
        for c4 in range(4):
            for hl in range(8 * c4, 8 * c4 + 8):
                inv_row(b, hl)
            o_cp(b * 4 + c4).start()

    w_cp.start()
    z_ref[...] = jnp.zeros(z_ref.shape, u32)
    w_cp.wait()
    h_cp.start()
    x_cp(0).start()
    w_prep()
    for f in range(2):
        for k in range(NT * 6):
            wgen_piece(f, k)
    h_cp.wait()
    x_cp(1).start()
    fwd_rows(xh_ref, 0, 4, 0, True)
    x_cp(0).wait()
    for b in range(2, NB):
        x_cp(b).start()
    fwd_block(0)

    main_slot(0, NC)
    for f in range(1, 9):
        for half, s in enumerate((f - 1, 16 - f)):
            side = None
            if f < 8:
                side = lambda i, f=f, half=half: [wgen_piece(f + 1, 27 * half + 3 * i + r) for r in range(3)]
            main_slot(0, s, side)
    x_cp(1).wait()
    fwd_block(1)
    inv_block(0)

    @pl.loop(1, NB - 1)
    def _(b):
        main_block(b)
        x_cp(b + 1).wait()
        fwd_block(b + 1)
        inv_block(b)

    main_block(NB - 1)
    inv_block(NB - 1)
    for c in range(NB * 4):
        o_cp(c).wait()


@jax.jit
def pallas_standalone__fft_conv__vision_kernel(x: jax.Array, w: jax.Array):
    x3 = x.reshape(H, W, C).transpose(0, 2, 1)
    w3 = w.reshape(49, C, C)
    y = pl.pallas_call(
        _kernel,
        in_specs=[
            pl.BlockSpec(memory_space=pl.ANY),
            pl.BlockSpec(memory_space=pl.ANY),
            pl.BlockSpec(memory_space=pltpu.VMEM),
            pl.BlockSpec(memory_space=pltpu.VMEM),
        ],
        out_specs=pl.BlockSpec(memory_space=pl.ANY),
        out_shape=jax.ShapeDtypeStruct((H, C, W), bf16),
        scratch_shapes=[
            pltpu.VMEM((9 * NC * PR, 128), u32),
            pltpu.VMEM((6 * PR + 4, 128), u32),
            pltpu.VMEM((NS * 3 * NT, C // 2, 128), u32),
            pltpu.VMEM((NT * 7, C, 128), f32),
            pltpu.VMEM((HB * 8 * ZR, 128), u32),
            pltpu.VMEM((2, 136, 128), f32),
            pltpu.VMEM((H, C, W), bf16),
            pltpu.VMEM((8, C, W), bf16),
            pltpu.VMEM((49, C, C), bf16),
            pltpu.VMEM((H, C, W), bf16),
            pltpu.SemaphoreType.DMA((NB + 2,)),
            pltpu.SemaphoreType.DMA((NB * 4,)),
        ],
        compiler_params=pltpu.CompilerParams(vmem_limit_bytes=110 * 2**20),
    )(x3, w3, jnp.asarray(_F), jnp.asarray(_G))
    return y.transpose(0, 2, 1).reshape(1, H, W, C)
```

```python
import numpy as np
import jax
import jax.numpy as jnp
from jax import lax
import jax.experimental.pallas as pl
import jax.experimental.pallas.tpu as pltpu

H = W = 224
C = 96
T = 34
V = 28
NC = 16
NS = 17
HB = 32
JB = HB // 2
NB = H // HB
PR = 4 * (4 + H // 2) + 4
ZR = 20
NT = 9

bf16 = jnp.bfloat16
f32 = jnp.float32
u32 = jnp.uint32


def _round_bf16(m):
    b = np.ascontiguousarray(m, np.float32).view(np.uint32).astype(np.uint64)
    b = ((b + 0x7FFF + ((b >> 16) & 1)) >> 16) << 16
    return b.astype(np.uint32).view(np.float32)


def _consts():
    fm = np.zeros((2, 136, 128), np.float64)
    gm = np.zeros((2 * V, 128), np.float64)
    for u in range(2):
        wl = [l if l < 112 else l + 96 for l in range(128)] if u == 0 else \
             [128 + l if l < 96 else l for l in range(128)]
        for tl in range(4):
            for l in range(128):
                n = (wl[l] - (V * (4 * u + tl) - 6)) % W
                if n >= T:
                    continue
                for s in range(NC):
                    ph = 2 * np.pi * (s + 1) * n / T
                    fm[u, tl * 16 + s, l] = np.cos(ph)
                    fm[u, 64 + tl * 16 + s, l] = -np.sin(ph)
                r = 128 + 4 * (tl % 2) + tl // 2
                fm[u, r, l] = 1.0
                fm[u, r + 2, l] = (-1.0) ** n
    for tl in range(2):
        for m in range(V):
            n = m + 6 - 3
            r, c = tl * V + m, tl * 2 * ZR
            for s in range(NC):
                ph = 2 * np.pi * (s + 1) * n / T
                gm[r, c + 2 * s] = 2 * np.cos(ph) / T
                gm[r, c + 2 * s + 1] = -2 * np.sin(ph) / T
            gm[r, c + 2 * NC] = (-1.0) ** n / T
            gm[r, c + 2 * NC + 1] = 1.0 / T
    return _round_bf16(fm), _round_bf16(gm)


_F, _G = _consts()
_COS = [[float(np.cos(2 * np.pi * f * k / T)) for k in range(4)] for f in range(9)]
_SIN = [[float(np.sin(2 * np.pi * f * k / T)) for k in range(4)] for f in range(9)]
_NT_DIMS = (((1,), (1,)), ((), ()))
_NN_DIMS = (((1,), (0,)), ((), ()))


def _pk(lo, hi):
    return pltpu.pack_elementwise([lo, hi], packed_dtype=bf16)


def _kernel(x_hbm, w_hbm, f_ref, g_ref, o_hbm,
            p_ref, pr_ref, wt_ref, sd_ref, z_ref, rp_ref, xb_ref, xh_ref, w_ref, ob_ref, isem, osem):
    w_cp = pltpu.make_async_copy(w_hbm, w_ref, isem.at[NB])
    h_cp = pltpu.make_async_copy(x_hbm.at[pl.ds(H - 8, 8)], xh_ref, isem.at[NB + 1])

    def x_cp(b):
        return pltpu.make_async_copy(x_hbm.at[pl.ds(b * HB, HB)], xb_ref.at[pl.ds(b * HB, HB)], isem.at[b])

    def o_cp(c):
        return pltpu.make_async_copy(ob_ref.at[pl.ds(c * 8, 8)], o_hbm.at[pl.ds(c * 8, 8)], osem.at[0])

    def dft(xrow, u):
        xr = xrow[...]
        if u == 0:
            win = jnp.concatenate([xr[:, 0:112], xr[:, 208:224]], axis=1)
        else:
            win = jnp.concatenate([xr[:, 128:224], xr[:, 96:128]], axis=1)
        win = jnp.concatenate([win, jnp.zeros((128 - C, 128), bf16)], axis=0)
        return lax.dot_general(f_ref[u], win, _NT_DIMS, preferred_element_type=f32)

    def emit(r, m, row):
        for pp in range(2):
            b0, b1 = r[32 * pp:32 * pp + 16], r[32 * pp + 16:32 * pp + 32]
            c0, c1 = r[64 + 32 * pp:80 + 32 * pp], r[80 + 32 * pp:96 + 32 * pp]
            for g, v in enumerate((_pk(b0 + c0, b1 + c1), _pk(b0, b1), _pk(c0, c1))):
                p_ref[pl.ds((m * 3 + g) * NC * PR + row + pp, NC, stride=PR), :] = v
        rr = _pk(r[128:136], pltpu.roll(r[128:136], 4, 0))
        for c in range(2):
            pr_ref[pl.ds((m * 2 + c) * PR + row, 2), :] = rr[2 * c:2 * c + 2]

    def fwd_rows(src, h0, npairs, row0, first):
        for u in range(2):
            prev = None if first else rp_ref[u]
            for jj in range(npairs):
                r0 = dft(src.at[h0 + 2 * jj], u)
                r1 = dft(src.at[h0 + 2 * jj + 1], u)
                row = row0 + 4 * jj + 2 * u
                emit(r0, 0, row)
                emit(r1 - r0, 1, row)
                if prev is not None:
                    emit(r0 - prev, 2, row)
                prev = r1
            rp_ref[u] = prev

    def fwd_block(b):
        fwd_rows(xb_ref, b * HB, JB, b * (4 * JB) + 16, False)

    def w_prep():
        for kw in range(7):
            ws = [w_ref[p * 7 + kw].astype(f32) for p in range(7)]
            tiles = []
            for sq in ([ws[0] + ws[1], ws[2] + ws[3], ws[4] + ws[5], ws[6]], [ws[0], ws[2], ws[4], ws[6]]):
                d = jnp.concatenate(sq, axis=0)
                tiles += [d[128 * k:128 * (k + 1)] for k in range(3)]
            for q in range(3):
                tiles.append(jnp.concatenate([-ws[2 * q + 1], jnp.zeros((128 - C, C), f32)], axis=0))
            for k, v in enumerate(tiles):
                v = jnp.concatenate([v, jnp.zeros((128, 128 - C), f32)], axis=1)
                sd_ref[k * 7 + kw] = v.T[:C]
        for tp in range(NT):
            t_ = [sd_ref[tp * 7 + k] for k in range(7)]
            sd_ref[tp * 7] = t_[3]
            for k in range(1, 4):
                sd_ref[tp * 7 + k] = t_[3 + k] + t_[3 - k]
                sd_ref[tp * 7 + 3 + k] = t_[3 + k] - t_[3 - k]

    def wgen_piece(f, k):
        tp, og = k // 6, k % 6
        outs = []
        for par in range(2):
            rows = pl.ds(16 * og + par, 8, stride=2)
            if f == 0:
                w0, s1, s2, s3 = [sd_ref[tp * 7 + i, rows, :] for i in range(4)]
                e, o = w0 + s2, s1 + s3
                outs.append((e + o, e - o))
                continue
            w0, s1, s2, s3, d1, d2, d3 = [sd_ref[tp * 7 + i, rows, :] for i in range(7)]
            cs, sn = _COS[f], _SIN[f]
            a, b = w0 + s2 * cs[2], s1 * cs[1] + s3 * cs[3]
            cc, dd = d2 * (-sn[2]), d1 * (-sn[1]) + d3 * (-sn[3])
            wr0, wr1, wi0, wi1 = a + b, a - b, cc + dd, dd - cc
            outs.append((wr0, wi0 - wr0, wr0 + wi0, wr1, wi1 - wr1, wr1 + wi1))
        dst = ((NC, 1), (NC, 2)) if f == 0 else \
              ((f - 1, 0), (f - 1, 1), (f - 1, 2), (16 - f, 0), (16 - f, 1), (16 - f, 2))
        for i, (s, g) in enumerate(dst):
            wt_ref[(s * 3 + g) * NT + tp, pl.ds(8 * og, 8), :] = _pk(outs[0][i], outs[1][i])

    def prod(src, sb, wb, m):
        lane = lax.broadcasted_iota(jnp.int32, (4 * JB, 128), 1)
        ld = lambda q: src[pl.ds(sb - 4 * q, 4 * JB), :]
        if m < 2:
            r1, r2, r3 = pltpu.roll(ld(1), 96, 1), pltpu.roll(ld(2), 64, 1), pltpu.roll(ld(3), 32, 1)
            parts = [jnp.where(lane < 96, ld(0), r1), jnp.where(lane < 64, r1, r2), jnp.where(lane < 32, r2, r3)]
        else:
            parts = [ld(0), ld(1), ld(2)]
        rhs = jnp.concatenate([pltpu.bitcast(v, bf16) for v in parts], axis=1)
        lhs = jnp.concatenate([pltpu.bitcast(wt_ref[wb + 3 * m + q], bf16) for q in range(3)], axis=1)
        return lax.dot_general(lhs, rhs, _NT_DIMS, preferred_element_type=f32)

    def put_z(yr, yi, e, s):
        zt = jnp.concatenate([_pk(yr, yi), jnp.zeros((128 - C, 128), u32)], axis=0).T
        for j in range(JB):
            z_ref[pl.ds((2 * j + e) * 8 * ZR + s, 8, stride=ZR), :] = zt[8 * j:8 * j + 8]

    def main_slot(b, s, side=None):
        base = b * (4 * JB) + 16
        ms = []
        for m in range(3):
            if s < NC:
                k = []
                for g in range(3):
                    k.append(prod(p_ref, ((m * 3 + g) * NC + s) * PR + base, (s * 3 + g) * NT, m))
                    if side is not None:
                        side(m * 3 + g)
                ms.append((k[0] - k[2], k[0] + k[1]))
            else:
                ms.append((prod(pr_ref, (m * 2 + 1) * PR + base, (s * 3 + 2) * NT, m),
                           prod(pr_ref, (m * 2) * PR + base, (s * 3 + 1) * NT, m)))
            if m == 1:
                put_z(ms[0][0] + ms[1][0], ms[0][1] + ms[1][1], 1, s)
        put_z(ms[0][0] + ms[2][0], ms[0][1] + ms[2][1], 0, s)

    def main_block(b):
        for s in range(NS):
            main_slot(b, s)

    def inv_row(b, hl):
        ys = []
        for q in range(4):
            zz = pltpu.bitcast(z_ref[pl.ds((hl * 8 + 2 * q) * ZR, 2 * ZR), :], bf16)
            zz = jnp.concatenate([zz, jnp.zeros((128 - 4 * ZR, 128), bf16)], axis=0)
            ys.append(lax.dot_general(g_ref[...], zz, _NN_DIMS, preferred_element_type=f32))
        y = jnp.concatenate(ys + [jnp.zeros((256 - W, 128), f32)], axis=0)
        ob_ref[b * HB + hl] = y.T[:C, :W].astype(bf16)

    def inv_block(b):
        for c4 in range(4):
            for hl in range(8 * c4, 8 * c4 + 8):
                inv_row(b, hl)
            o_cp(b * 4 + c4).start()

    h_cp.start()
    w_cp.start()
    z_ref[...] = jnp.zeros(z_ref.shape, u32)
    h_cp.wait()
    x_cp(0).start()
    fwd_rows(xh_ref, 0, 4, 0, True)
    w_cp.wait()
    w_prep()
    for f in range(2):
        for k in range(NT * 6):
            wgen_piece(f, k)
    x_cp(0).wait()
    for b in range(1, NB):
        x_cp(b).start()
    fwd_block(0)

    main_slot(0, NC)
    for f in range(1, 9):
        for half, s in enumerate((f - 1, 16 - f)):
            side = None
            if f < 8:
                side = lambda i, f=f, half=half: [wgen_piece(f + 1, 27 * half + 3 * i + r) for r in range(3)]
            main_slot(0, s, side)
    x_cp(1).wait()
    fwd_block(1)
    inv_block(0)

    @pl.loop(1, NB - 1)
    def _(b):
        x_cp(b + 1).wait()
        main_block(b)
        fwd_block(b + 1)
        inv_block(b)

    main_block(NB - 1)
    inv_block(NB - 1)
    pltpu.make_async_copy(ob_ref, o_hbm, osem.at[0]).wait()


@jax.jit
def pallas_standalone__fft_conv__vision_kernel(x: jax.Array, w: jax.Array):
    x3 = x.reshape(H, W, C).transpose(0, 2, 1)
    w3 = w.reshape(49, C, C)
    y = pl.pallas_call(
        _kernel,
        in_specs=[
            pl.BlockSpec(memory_space=pl.ANY),
            pl.BlockSpec(memory_space=pl.ANY),
            pl.BlockSpec(memory_space=pltpu.VMEM),
            pl.BlockSpec(memory_space=pltpu.VMEM),
        ],
        out_specs=pl.BlockSpec(memory_space=pl.ANY),
        out_shape=jax.ShapeDtypeStruct((H, C, W), bf16),
        scratch_shapes=[
            pltpu.VMEM((9 * NC * PR, 128), u32),
            pltpu.VMEM((6 * PR + 4, 128), u32),
            pltpu.VMEM((NS * 3 * NT, C // 2, 128), u32),
            pltpu.VMEM((NT * 7, C, 128), f32),
            pltpu.VMEM((HB * 8 * ZR, 128), u32),
            pltpu.VMEM((2, 136, 128), f32),
            pltpu.VMEM((H, C, W), bf16),
            pltpu.VMEM((8, C, W), bf16),
            pltpu.VMEM((49, C, C), bf16),
            pltpu.VMEM((H, C, W), bf16),
            pltpu.SemaphoreType.DMA((NB + 2,)),
            pltpu.SemaphoreType.DMA((1,)),
        ],
        compiler_params=pltpu.CompilerParams(vmem_limit_bytes=110 * 2**20, flags={'XLA_TPU_FORCE_LP_LLO_SCHEDULER': True}),
    )(x3, w3, jnp.asarray(_F), jnp.asarray(_G))
    return y.transpose(0, 2, 1).reshape(1, H, W, C)
```
